```python
import os as _os
_os.environ.setdefault("JAX_PLATFORMS", "cpu")
import jax
import jax.numpy as jnp

def _softmax(x, axis=-1):
    return jax.nn.softmax(x, axis=axis)
def _gelu(x):
    return jax.nn.gelu(x, approximate=True)
def _silu(x):
    return jax.nn.silu(x)
def _sigmoid(x):
    return jax.nn.sigmoid(x)
def _layernorm(x, axis=-1, eps=1e-5):
    m = jnp.mean(x, axis=axis, keepdims=True)
    v = jnp.var(x, axis=axis, keepdims=True)
    return (x - m) / jnp.sqrt(v + eps)
def _scatter_add(tgt, idx, src, axis=0):
    return tgt.at[idx].add(src)
def _segment_sum(src, seg, n):
    return jax.ops.segment_sum(src, seg, n)
class _Rng:
    def __init__(self, key):
        self._k = key
    def _next(self):
        self._k, sub = jax.random.split(self._k)
        return sub
    def normal(self, shape):
        return jax.random.normal(self._next(), shape, dtype=jnp.bfloat16)
    def randint(self, lo, hi, shape):
        return jax.random.randint(self._next(), shape, lo, hi, dtype=jnp.int32)
    def uniform(self, shape, lo=0.0, hi=1.0):
        return jax.random.uniform(self._next(), shape, jnp.bfloat16, lo, hi)
    def permutation(self, n):
        return jax.random.permutation(self._next(), n)


kernel_name = 'standalone__groupnorm__sampling'

def setup_inputs():
    _rng = _Rng(jax.random.key(int.from_bytes(__import__("os").urandom(4), "little")))
    _w = (lambda a: (lambda t: t.astype(jnp.bfloat16) if jnp.issubdtype(t.dtype, jnp.floating) else t)(jnp.asarray(a)))
    B = 32
    G = 32
    cpg = max(1, 576 // G)
    C = G * cpg
    H, W = 32, 16
    return {
        "x": _w((lambda *s: _rng.normal(s) * 0.05)(B, C, H, W)),
        "g": _w((lambda *s: _rng.normal(s) * 0.05)(C) + 1.0),
        "b": _w((lambda *s: _rng.normal(s) * 0.05)(C)),
    }

def reference(x, g, b):
    G = 32
    B, C, H, W = x.shape[0], x.shape[1], x.shape[2], x.shape[3]
    xr = x.reshape(B, G, C // G, H, W)
    mu = xr.mean(axis=(2, 3, 4), keepdims=True)
    var = ((xr - mu) ** 2).mean(axis=(2, 3, 4), keepdims=True)
    xn = (xr - mu) / jnp.sqrt(var + 1e-5)
    xn = xn.reshape(B, C, H, W)
    return xn * g[None, :, None, None] + b[None, :, None, None]
```

```python
import functools

import jax
import jax.numpy as jnp
from jax import lax
from jax.experimental import pallas as pl
from jax.experimental.pallas import tpu as pltpu

_GROUPS = 32
_EPS = 1e-5

_SLABS = 4
_TAIL_ROWS = 256
_WRITE_STRIDE = 816
_WRITE_CHUNK = 32
_TILE = 16


def _kernel(x_hbm, gamma_hbm, beta_hbm, o_hbm,
            x_buf, o_buf, gamma_buf, beta_buf, same_group, stats,
            read_sems, param_sems, write_sem, *, spatial):
  rows, channels = x_buf.shape
  per_group = channels // _GROUPS
  slab_rows = rows // _SLABS
  slab_batch = slab_rows // spatial

  def read(start, size, i):
    return pltpu.make_async_copy(
        x_hbm.at[pl.ds(start, size)], x_buf.at[pl.ds(start, size)],
        read_sems.at[i])

  bounds = [i * slab_rows for i in range(_SLABS)] + [rows - _TAIL_ROWS, rows]
  reads = [read(lo, hi - lo, i)
           for i, (lo, hi) in enumerate(zip(bounds[:-1], bounds[1:]))]
  for copy in reads:
    copy.start(priority=1)
  gamma_copy = pltpu.make_async_copy(gamma_hbm, gamma_buf, param_sems.at[0])
  beta_copy = pltpu.make_async_copy(beta_hbm, beta_buf, param_sems.at[1])
  gamma_copy.start()
  beta_copy.start()

  shift = 20
  inverse = -(-(1 << shift) // per_group)
  assert all((c * inverse) >> shift == c // per_group for c in range(channels))
  col_group = (
      lax.broadcasted_iota(jnp.int32, (_TILE, channels), 1) * inverse) >> shift

  def fill_same_group(i, _):
    r0 = pl.multiple_of(i * _TILE, _TILE)
    row = lax.broadcasted_iota(jnp.int32, (_TILE, channels), 0) + r0
    same = ((row * inverse) >> shift) == col_group
    same_group[pl.ds(r0, _TILE), :] = jnp.where(same, 1.0, 0.0).astype(
        same_group.dtype)

  lax.fori_loop(0, channels // _TILE, fill_same_group, None)

  def group_mean(col_sums):
    hi = col_sums.astype(jnp.bfloat16).astype(jnp.float32)
    rest = col_sums - hi
    mid = rest.astype(jnp.bfloat16).astype(jnp.float32)
    lo = rest - mid
    parts = jnp.concatenate([hi, mid, lo, jnp.zeros_like(lo)], axis=0)
    t = jnp.dot(parts.astype(jnp.bfloat16), same_group[...],
                preferred_element_type=jnp.float32)
    n = slab_batch
    return (t[:n] + (t[n:2 * n] + t[2 * n:3 * n])) * (1.0 / (spatial * per_group))

  gamma_copy.wait()
  beta_copy.wait()
  gamma = gamma_buf[...].astype(jnp.float32).reshape(1, channels)
  beta = beta_buf[...].astype(jnp.float32).reshape(1, channels)

  def tiles(slab_start, i):
    base = pl.multiple_of(slab_start + i * spatial, spatial)
    return [pl.ds(base + t, _TILE) for t in range(0, spatial, _TILE)]

  def per_row(values):
    return jnp.broadcast_to(values, (_TILE, channels))

  def normalize(slab_start):
    def sum_pass(i, _):
      acc = jnp.zeros((_TILE, channels), jnp.float32)
      for tile in tiles(slab_start, i):
        acc += x_buf[tile, :].astype(jnp.float32)
      stats[0, pl.ds(i, 1), :] = jnp.sum(acc, axis=0, keepdims=True)

    lax.fori_loop(0, slab_batch, sum_pass, None)
    stats[1] = group_mean(stats[0])

    def variance_pass(i, _):
      mean = per_row(stats[1, pl.ds(i, 1), :])
      acc = jnp.zeros((_TILE, channels), jnp.float32)
      for tile in tiles(slab_start, i):
        centered = x_buf[tile, :].astype(jnp.float32) - mean
        acc += centered * centered
      stats[0, pl.ds(i, 1), :] = jnp.sum(acc, axis=0, keepdims=True)

    lax.fori_loop(0, slab_batch, variance_pass, None)
    stats[2] = gamma * lax.rsqrt(group_mean(stats[0]) + _EPS)

    def output_pass(i, _):
      mean = per_row(stats[1, pl.ds(i, 1), :])
      scale = per_row(stats[2, pl.ds(i, 1), :])
      offset = per_row(beta)
      for tile in tiles(slab_start, i):
        centered = x_buf[tile, :].astype(jnp.float32) - mean
        o_buf[tile, :] = (centered * scale + offset).astype(o_buf.dtype)

    lax.fori_loop(0, slab_batch, output_pass, None)

  def write(slab_start):
    jumps = slab_rows // _WRITE_STRIDE
    strided_rows = jumps * _WRITE_STRIDE
    shape = (jumps, _WRITE_STRIDE, channels)
    src = o_buf.at[pl.ds(slab_start, strided_rows)].reshape(shape)
    dst = o_hbm.at[pl.ds(slab_start, strided_rows)].reshape(shape)

    def start(window):
      pltpu.make_async_copy(
          src.at[:, window], dst.at[:, window], write_sem).start()

    chunks, last = divmod(_WRITE_STRIDE, _WRITE_CHUNK)
    lax.fori_loop(
        0, chunks,
        lambda i, _: start(
            pl.ds(pl.multiple_of(i * _WRITE_CHUNK, _WRITE_CHUNK), _WRITE_CHUNK)),
        None)
    if last:
      start(pl.ds(chunks * _WRITE_CHUNK, last))
    if strided_rows < slab_rows:
      rest = pl.ds(slab_start + strided_rows, slab_rows - strided_rows)
      pltpu.make_async_copy(o_buf.at[rest], o_hbm.at[rest], write_sem).start()

  def slab(j, _):
    slab_start = pl.multiple_of(j * slab_rows, slab_rows)

    @pl.when(j < _SLABS - 1)
    def _():
      read(slab_start, slab_rows, j).wait()

    @pl.when(j == _SLABS - 1)
    def _():
      reads[-2].wait()
      write(0)
      reads[-1].wait()

    normalize(slab_start)

  lax.fori_loop(0, _SLABS, slab, None)
  lax.fori_loop(
      1, _SLABS,
      lambda j, _: write(pl.multiple_of(j * slab_rows, slab_rows)), None)
  pltpu.make_async_copy(o_buf, o_hbm, write_sem).wait()


@jax.jit
def pallas_standalone__groupnorm__sampling_kernel(
    x: jax.Array,
    g: jax.Array,
    b: jax.Array,
):
  batch, channels, height, width = x.shape
  rows = batch * height * width
  x_rows = jnp.transpose(x, (0, 2, 3, 1)).reshape(rows, channels)

  in_hbm = pl.BlockSpec(memory_space=pltpu.HBM)
  out = pl.pallas_call(
      functools.partial(_kernel, spatial=height * width),
      in_specs=[in_hbm, in_hbm, in_hbm],
      out_specs=in_hbm,
      out_shape=jax.ShapeDtypeStruct((rows, channels), x.dtype),
      scratch_shapes=[
          pltpu.VMEM((rows, channels), x.dtype),
          pltpu.VMEM((rows, channels), x.dtype),
          pltpu.VMEM((channels,), g.dtype),
          pltpu.VMEM((channels,), b.dtype),
          pltpu.VMEM((channels, channels), jnp.bfloat16),
          pltpu.VMEM((3, batch // _SLABS, channels), jnp.float32),
          pltpu.SemaphoreType.DMA((_SLABS + 1,)),
          pltpu.SemaphoreType.DMA((2,)),
          pltpu.SemaphoreType.DMA,
      ],
      compiler_params=pltpu.CompilerParams(
          vmem_limit_bytes=64 * 1024 * 1024,
          disable_bounds_checks=True,
          disable_semaphore_checks=True,
      ),
  )(x_rows, g, b)
  return jnp.transpose(
      out.reshape(batch, height, width, channels), (0, 3, 1, 2))
```

```python
import functools

import jax
import jax.numpy as jnp
from jax import lax
from jax.experimental import pallas as pl
from jax.experimental.pallas import tpu as pltpu

_GROUPS = 32
_EPS = 1e-5

_TILE = 16
_SLABS = 4
_TAIL_ROWS = 288
_EARLY_STREAMS = (5, 6)
_LATE_STREAMS = (5,)
_WRITE_CHUNK = 24


def _group_mean(channel_sums, count):
  channels = channel_sums.shape[1]
  per_group = channels // _GROUPS
  channel = lax.broadcasted_iota(jnp.int32, channel_sums.shape, 1)
  total = jnp.zeros_like(channel_sums)
  for first in range(0, channels, per_group):
    member = (channel >= first) & (channel < first + per_group)
    group_sum = jnp.sum(
        jnp.where(member, channel_sums, 0.0), axis=1, keepdims=True)
    total = jnp.where(member, group_sum, total)
  return total / count


def _normalize(x_buf, o_buf, stats, gamma, beta, slab, spatial):
  _, slab_batch, channels = stats.shape
  count = spatial * (channels // _GROUPS)
  per_block = o_buf.shape[1] // spatial
  offsets = range(0, spatial, _TILE)

  def load_tiles(i):
    base = pl.multiple_of((slab * slab_batch + i) * spatial, spatial)
    for t in offsets:
      yield x_buf[pl.ds(base + t, _TILE), :].astype(jnp.float32)

  def per_row(values):
    return jnp.broadcast_to(values, (_TILE, channels))

  def sum_pass(i, _):
    acc = jnp.zeros((_TILE, channels), jnp.float32)
    for x in load_tiles(i):
      acc += x
    stats[0, pl.ds(i, 1), :] = jnp.sum(acc, axis=0, keepdims=True)

  lax.fori_loop(0, slab_batch, sum_pass, None)
  stats[1] = _group_mean(stats[0], count)

  def variance_pass(i, _):
    mean = per_row(stats[1, pl.ds(i, 1), :])
    acc = jnp.zeros((_TILE, channels), jnp.float32)
    for x in load_tiles(i):
      centered = x - mean
      acc += centered * centered
    stats[0, pl.ds(i, 1), :] = jnp.sum(acc, axis=0, keepdims=True)

  lax.fori_loop(0, slab_batch, variance_pass, None)
  stats[2] = gamma * lax.rsqrt(_group_mean(stats[0], count) + _EPS)

  def output_pass(i, _):
    mean = per_row(stats[1, pl.ds(i, 1), :])
    scale = per_row(stats[2, pl.ds(i, 1), :])
    shift = per_row(beta)
    element = slab * slab_batch + i
    block = lax.div(element, per_block)
    base = pl.multiple_of(lax.rem(element, per_block) * spatial, spatial)
    for t, x in zip(offsets, load_tiles(i)):
      y = (x - mean) * scale + shift
      o_buf[block, pl.ds(base + t, _TILE), :] = y.astype(o_buf.dtype)

  lax.fori_loop(0, slab_batch, output_pass, None)


def _kernel(x_hbm, gamma_hbm, beta_hbm, o_hbm,
            x_buf, o_buf, gamma_buf, beta_buf, stats, write_sem, *, spatial):
  rows, channels = x_buf.shape
  block_rows = o_buf.shape[1]
  slab_rows = rows // _SLABS
  assert sum(_EARLY_STREAMS) * block_rows <= rows - slab_rows

  def start_writes(first_block, stream_counts):
    turns, last = divmod(block_rows, _WRITE_CHUNK)
    for streams in stream_counts:
      blocks = pl.ds(first_block, streams)
      first_block += streams

      def start(chunk, blocks=blocks):
        pltpu.make_async_copy(
            o_buf.at[blocks, chunk], o_hbm.at[blocks, chunk], write_sem).start()

      def turn(i, _, start=start):
        start(pl.ds(pl.multiple_of(i * _WRITE_CHUNK, _WRITE_CHUNK),
                    _WRITE_CHUNK))

      lax.fori_loop(0, turns, turn, None)
      if last:
        start(pl.ds(turns * _WRITE_CHUNK, last))

  def read_and_normalize(read_sems, param_sem):
    def read(first_row, size, i):
      span = pl.ds(first_row, size)
      return pltpu.make_async_copy(
          x_hbm.at[span], x_buf.at[span], read_sems.at[i])

    bounds = [i * slab_rows for i in range(_SLABS)] + [rows - _TAIL_ROWS, rows]
    reads = [read(lo, hi - lo, i)
             for i, (lo, hi) in enumerate(zip(bounds[:-1], bounds[1:]))]
    params = [pltpu.make_async_copy(gamma_hbm, gamma_buf, param_sem),
              pltpu.make_async_copy(beta_hbm, beta_buf, param_sem)]
    for copy in reads:
      copy.start(priority=1)
    for copy in params:
      copy.start()
    for copy in params:
      copy.wait()
    gamma = gamma_buf[...].astype(jnp.float32).reshape(1, channels)
    beta = beta_buf[...].astype(jnp.float32).reshape(1, channels)

    def process(slab, _):
      @pl.when(slab < _SLABS - 1)
      def _():
        read(pl.multiple_of(slab * slab_rows, slab_rows), slab_rows, slab).wait()

      @pl.when(slab == _SLABS - 1)
      def _():
        reads[-2].wait()
        start_writes(0, _EARLY_STREAMS)
        reads[-1].wait()

      _normalize(x_buf, o_buf, stats, gamma, beta, slab, spatial)

    lax.fori_loop(0, _SLABS, process, None)

  pl.run_scoped(read_and_normalize,
                pltpu.SemaphoreType.DMA((_SLABS + 1,)),
                pltpu.SemaphoreType.DMA(()))

  start_writes(sum(_EARLY_STREAMS), _LATE_STREAMS)
  pltpu.make_async_copy(o_buf, o_hbm, write_sem).wait()


@jax.jit
def pallas_standalone__groupnorm__sampling_kernel(
    x: jax.Array,
    g: jax.Array,
    b: jax.Array,
):
  batch, channels, height, width = x.shape
  rows = batch * height * width
  blocks = sum(_EARLY_STREAMS) + sum(_LATE_STREAMS)
  assert batch % blocks == 0 and batch % _SLABS == 0
  out_shape = (blocks, rows // blocks, channels)
  x_rows = jnp.transpose(x, (0, 2, 3, 1)).reshape(rows, channels)

  in_hbm = pl.BlockSpec(memory_space=pltpu.HBM)
  out = pl.pallas_call(
      functools.partial(_kernel, spatial=height * width),
      in_specs=[in_hbm, in_hbm, in_hbm],
      out_specs=in_hbm,
      out_shape=jax.ShapeDtypeStruct(out_shape, x.dtype),
      scratch_shapes=[
          pltpu.VMEM((rows, channels), x.dtype),
          pltpu.VMEM(out_shape, x.dtype),
          pltpu.VMEM((channels,), g.dtype),
          pltpu.VMEM((channels,), b.dtype),
          pltpu.VMEM((3, batch // _SLABS, channels), jnp.float32),
          pltpu.SemaphoreType.DMA,
      ],
      compiler_params=pltpu.CompilerParams(vmem_limit_bytes=64 * 1024 * 1024),
  )(x_rows, g, b)
  return jnp.transpose(
      out.reshape(batch, height, width, channels), (0, 3, 1, 2))
```
